```python
import jax
import jax.numpy as jnp

def _softmax(x, axis=-1):
    return jax.nn.softmax(x, axis=axis)

def _gelu(x):
    return jax.nn.gelu(x, approximate=True)

def _silu(x):
    return jax.nn.silu(x)

def _sigmoid(x):
    return jax.nn.sigmoid(x)

def _layernorm(x, axis=-1, eps=1e-05):
    m = jnp.mean(x, axis=axis, keepdims=True)
    v = jnp.var(x, axis=axis, keepdims=True)
    return (x - m) / jnp.sqrt(v + eps)

def _scatter_add(tgt, idx, src, axis=0):
    return tgt.at[idx].add(src)

def _segment_sum(src, seg, n):
    return jax.ops.segment_sum(src, seg, n)

class _Rng:

    def __init__(self, key):
        self._k = key

    def _next(self):
        self._k, sub = jax.random.split(self._k)
        return sub

    def normal(self, shape):
        return jax.random.normal(self._next(), shape, dtype=jnp.bfloat16)

    def randint(self, lo, hi, shape):
        return jax.random.randint(self._next(), shape, lo, hi, dtype=jnp.int32)

    def uniform(self, shape, lo=0.0, hi=1.0):
        return jax.random.uniform(self._next(), shape, jnp.bfloat16, lo, hi)

    def permutation(self, n):
        return jax.random.permutation(self._next(), n)
kernel_name = 'recurrent_scan__memory_aug_recurrent_mem_tr__glu_gated_glu__prompt'

def setup_inputs():
    _rng = _Rng(jax.random.key(int.from_bytes(__import__("os").urandom(4), "little")))
    _w = lambda a: (lambda t: t.astype(jnp.bfloat16) if jnp.issubdtype(t.dtype, jnp.floating) else t)(jnp.asarray(a))

    def _A_setup():
        B, S, Dm = (1, 2048, 1024)
        H, Dh = (32, 128)
        M, seg = (8, 32)
        seg = min(seg, S)
        S = S // seg * seg
        return {'x': _w((lambda *s: _rng.normal(s) * 0.05)(B, S, Dm)), 'mem0': _w((lambda *s: _rng.normal(s) * 0.05)(B, M, Dm)), 'Wq': _w((lambda *s: _rng.normal(s) * 0.05)(Dm, H, Dh) * Dm ** (-0.5)), 'Wk': _w((lambda *s: _rng.normal(s) * 0.05)(Dm, H, Dh) * Dm ** (-0.5)), 'Wv': _w((lambda *s: _rng.normal(s) * 0.05)(Dm, H, Dh) * Dm ** (-0.5)), 'Wo': _w((lambda *s: _rng.normal(s) * 0.05)(H, Dh, Dm) * (H * Dh) ** (-0.5)), 'seg_len': seg}
    _A_in = _A_setup()

    def _B_setup():
        B, S, D, F = (1, 2048, 1024, 3584)
        return {'x': _w((lambda *s: _rng.normal(s) * 0.05)(B, S, D)), 'w_gate': _w((lambda *s: _rng.normal(s) * 0.05)(D, F)), 'w_up': _w((lambda *s: _rng.normal(s) * 0.05)(D, F)), 'w_down': _w((lambda *s: _rng.normal(s) * 0.05)(F, D))}
    _B_in = _B_setup()
    return {'A_x': _A_in['x'], 'A_mem0': _A_in['mem0'], 'A_Wq': _A_in['Wq'], 'A_Wk': _A_in['Wk'], 'A_Wv': _A_in['Wv'], 'A_Wo': _A_in['Wo'], 'A_seg_len': _A_in['seg_len'], 'B_x': _B_in['x'], 'B_w_gate': _B_in['w_gate'], 'B_w_up': _B_in['w_up'], 'B_w_down': _B_in['w_down']}

def reference(A_x, A_mem0, A_Wq, A_Wk, A_Wv, A_Wo, A_seg_len, B_x, B_w_gate, B_w_up, B_w_down):

    def _A_ref(x, mem0, Wq, Wk, Wv, Wo, seg_len):
        B, S, Dm = x.shape
        H, Dh = (Wq.shape[1], Wq.shape[2])
        M = mem0.shape[1]
        scale = Dh ** (-0.5)
        n_seg = S // seg_len
        L = M + seg_len
        idx = jnp.arange(L)
        mask = (idx[:, None] < M) | (idx[:, None] >= idx[None, :])
        mem = mem0
        outs = []
        for s in range(n_seg):
            xs = x[:, s * seg_len:(s + 1) * seg_len, :].copy()
            h = jnp.concatenate([mem, xs], axis=1)
            q = jnp.einsum('btd,dhe->bhte', h, Wq)
            k = jnp.einsum('btd,dhe->bhte', h, Wk)
            v = jnp.einsum('btd,dhe->bhte', h, Wv)
            scores = jnp.einsum('bhqe,bhke->bhqk', q, k) * scale
            scores = jnp.where(mask[None, None], scores, -1000000000.0)
            p = _softmax(scores, axis=-1)
            o = jnp.einsum('bhqk,bhke->bhqe', p, v)
            o = jnp.einsum('bhte,hed->btd', o, Wo)
            mem = o[:, :M, :].copy()
            outs.append(o[:, M:, :])
        return jnp.concatenate(outs, axis=1)

    def _B_ref(x, w_gate, w_up, w_down):
        g = jnp.einsum('bsd,df->bsf', x, w_gate)
        u = jnp.einsum('bsd,df->bsf', x, w_up)
        h = _sigmoid(g) * u
        return jnp.einsum('bsf,fd->bsd', h, w_down)
    x = A_x
    xn = _layernorm(x, axis=-1)
    s = _A_ref(xn, A_mem0, A_Wq, A_Wk, A_Wv, A_Wo, A_seg_len)
    g = _silu(_B_ref(xn, B_w_gate, B_w_up, B_w_down))
    return x + s * g
```

```python
import functools

import jax
import jax.numpy as jnp
import jax.experimental.pallas as pl
import jax.experimental.pallas.tpu as pltpu

_PB = 128
_NPB = 6
_NJ = 4
_NCH = 16
_NSTG = 4
_LAG = 3
_NOB = 4
_SK1, _SK2 = 1, 2


def _kernel(x_hbm, mem0_ref, wq_hbm, wk_hbm, wv_hbm, wo_hbm, wg_hbm, wu_hbm, wd_hbm,
            out_hbm,
            wqkv, wo_i, wg, wu, wd, xv, xn, stg, stg2, h40, o40, sbuf, bacc, obuf,
            sem_b, sem_x, sem_s, sem_o,
            *, S, D, H, E, M, SEG, F):
    f32, bf16, u32 = jnp.float32, jnp.bfloat16, jnp.uint32
    L = M + SEG
    nseg = S // SEG
    FS = F // _NJ
    D2 = D // 2
    scale = E ** (-0.5)
    P = _PB * _NPB
    MB = (S - P) // (nseg // _NJ)
    DC = D // _NCH
    OC = H * E // _NCH
    dn = (((1,), (0,)), ((), ()))

    def b_copies(j):
        return [
            pltpu.make_async_copy(wg_hbm.at[:, pl.ds(j * FS, FS)], wg.at[j], sem_b.at[3 * j]),
            pltpu.make_async_copy(wu_hbm.at[:, pl.ds(j * FS, FS)], wu.at[j], sem_b.at[3 * j + 1]),
            pltpu.make_async_copy(wd_hbm.at[pl.ds(j * FS, FS), :], wd.at[j], sem_b.at[3 * j + 2]),
        ]

    def a_copies(c, slot):
        cps = []
        for j, src in enumerate((wq_hbm, wk_hbm, wv_hbm)):
            cps.append(pltpu.make_async_copy(src.at[pl.ds(pl.multiple_of(c * DC * H, DC * H), DC * H), :],
                                             stg.at[slot, j], sem_s.at[slot, j]))
        cps.append(pltpu.make_async_copy(wo_hbm.at[pl.ds(pl.multiple_of(c * OC, OC), OC), :],
                                         stg2.at[slot], sem_s.at[slot, 3]))
        return cps

    x_cp = pltpu.make_async_copy(x_hbm, xv, sem_x)
    x_cp.start()
    for cp in b_copies(0):
        cp.start()

    x_cp.wait()

    def ln(i, carry):
        r = pl.ds(pl.multiple_of(i * 64, 64), 64)
        xf = xv[r, :].astype(f32)
        m = jnp.mean(xf, axis=-1, keepdims=True)
        xc = xf - m
        v = jnp.mean(xc * xc, axis=-1, keepdims=True)
        xn[r, :] = xc * jax.lax.rsqrt(v + 1e-5)
        return carry

    jax.lax.fori_loop(0, S // 64, ln, 0)

    def glu_chunk(rows, js, fillers=()):
        fillers = list(fillers)
        nslot = 6
        per = -(-len(fillers) // nslot)

        def fill():
            for _ in range(min(per, len(fillers))):
                fillers.pop(0)()

        xb = xn[rows, :]
        c0 = (FS // E // 2 + 1) * E
        parts = ((0, c0), (c0, FS))
        hs = []
        gs = []
        for lo, hi in parts:
            gs.append(jax.lax.dot_general(xb, wg[js, :, lo:hi], dn, preferred_element_type=f32))
            fill()
        for (lo, hi), g in zip(parts, gs):
            u = jax.lax.dot_general(xb, wu[js, :, lo:hi], dn, preferred_element_type=f32)
            hs.append(jax.nn.sigmoid(g) * u)
            fill()
        d = None
        for (lo, hi), hb in zip(parts, hs):
            dd = jax.lax.dot_general(hb, wd[js, lo:hi, :], dn, preferred_element_type=f32)
            d = dd if d is None else d + dd
            fill()
        bacc[rows, :] = d + jnp.where(js > 0, bacc[rows, :], 0.0)

    def relayout_units(c, slot):
        sub = jax.lax.broadcasted_iota(jnp.int32, (8, E), 0)

        def tr8(vs):
            vs = list(vs)
            for k in (1, 2, 4):
                m = (sub & k) == 0
                for i in range(8):
                    if i & k == 0:
                        a, b = vs[i], vs[i + k]
                        vs[i] = jnp.where(m, a, pltpu.roll(b, k, 0))
                        vs[i + k] = jnp.where(m, pltpu.roll(a, 8 - k, 0), b)
            return vs

        def qkv_unit(j, g, half):
            los, his = [], []
            for dp in range(8):
                r0 = (g * 16 + dp * 2) * H + half * 16
                a = pltpu.bitcast(stg[slot, j, pl.ds(r0, 16), :], u32)
                b = pltpu.bitcast(stg[slot, j, pl.ds(r0 + H, 16), :], u32)
                los.append((a & u32(0xFFFF)) | (b << 16))
                his.append((a >> 16) | (b & u32(0xFFFF0000)))
            los, his = tr8(los), tr8(his)
            for hp in range(8):
                h = half * 16 + 2 * hp
                base = (h * 3 + j) * D2 + g * 8
                wqkv[pl.ds(pl.multiple_of(base + c * (DC // 2), 8), 8), :] = los[hp]
                wqkv[pl.ds(pl.multiple_of(base + 3 * D2 + c * (DC // 2), 8), 8), :] = his[hp]

        def wo_unit(r):
            v = stg2[slot, pl.ds(r * 16, 16), :]
            wo_i[pl.ds(pl.multiple_of(c * (OC // 2) + r * 8, 8), 8), :] = pltpu.bitcast(v, u32)

        units = []
        for j in range(3):
            for g in range(DC // 16):
                for half in range(H // 16):
                    units.append(functools.partial(qkv_unit, j, g, half))
        for r in range(OC // 16):
            units.append(functools.partial(wo_unit, r))
        return units

    n_pro = _NPB * _NJ
    n_plain = n_pro - _NCH

    def wait_b(i):
        @pl.when(i % _NPB == 0)
        def _():
            for cp in b_copies(i // _NPB):
                cp.wait()

            @pl.when(i // _NPB + 1 < _NJ)
            def _():
                for cp in b_copies(i // _NPB + 1):
                    cp.start()

        @pl.when(i == 0)
        def _():
            for c in range(_NSTG):
                for cp in a_copies(c, c):
                    cp.start()

    def pro_plain(i, carry):
        wait_b(i)
        glu_chunk(pl.ds(pl.multiple_of((i % _NPB) * _PB, _PB), _PB), i // _NPB)
        return carry

    def pro_relayout(i, carry):
        wait_b(i)
        c = i - n_plain
        slot = c % _NSTG
        for cp in a_copies(c, slot):
            cp.wait()
        glu_chunk(pl.ds(pl.multiple_of((i % _NPB) * _PB, _PB), _PB), i // _NPB, relayout_units(c, slot))

        @pl.when(c + _NSTG < _NCH)
        def _():
            for cp in a_copies(c + _NSTG, slot):
                cp.start()
        return carry

    jax.lax.fori_loop(0, n_plain, pro_plain, 0)
    jax.lax.fori_loop(n_plain, n_pro, pro_relayout, 0)

    h40[0:M, :] = mem0_ref[...].astype(f32)

    row = jax.lax.broadcasted_iota(jnp.int32, (L, L), 0)
    col = jax.lax.broadcasted_iota(jnp.int32, (L, L), 1)
    mask = (row < M) | (row >= col)

    def out_copy(sp, slot):
        return pltpu.make_async_copy(obuf.at[slot], out_hbm.at[pl.ds(pl.multiple_of(sp * SEG, SEG), SEG), :],
                                     sem_o.at[slot])

    def finalize(sp, slot):
        rows = pl.ds(pl.multiple_of(sp * SEG, SEG), SEG)
        b = bacc[rows, :]
        s_att = sbuf[pl.ds(pl.multiple_of((sp % 4) * SEG, SEG), SEG), :]
        obuf[slot] = (xv[rows, :].astype(f32) + s_att * (b * jax.nn.sigmoid(b))).astype(obuf.dtype)

    def step(s, carry):
        sp = jnp.maximum(s - _LAG, 0)
        slot = sp % _NOB

        @pl.when(s >= _LAG + _NOB)
        def _():
            out_copy(sp - _NOB, slot).wait()

        h40[M:L, :] = xn[pl.ds(pl.multiple_of(s * SEG, SEG), SEG), :]
        hh = h40[...]

        def proj(h, j):
            w = pltpu.bitcast(wqkv[(h * 3 + j) * D2:(h * 3 + j + 1) * D2, :], bf16)
            return jax.lax.dot_general(hh, w, dn, preferred_element_type=f32)

        def wo_part(i):
            n = H * E // 4
            return jax.lax.dot_general(o40[:, i * n:(i + 1) * n],
                                       pltpu.bitcast(wo_i[i * n // 2:(i + 1) * n // 2, :], bf16),
                                       dn, preferred_element_type=f32)

        qs, ks, vs, es, ls = {}, {}, {}, {}, {}
        r = None
        for t in range(H + _SK2):
            if t < H:
                qs[t] = proj(t, 0)
            h = t - _SK1
            if 0 <= h < H:
                sc = jax.lax.dot_general(qs.pop(h), ks.pop(h), (((1,), (1,)), ((), ())),
                                         preferred_element_type=f32) * scale
                sc = jnp.where(mask, sc, -1e9)
                e = jnp.exp(sc - jnp.max(sc, axis=-1, keepdims=True))
                es[h] = e
                ls[h] = 1.0 / jnp.sum(e, axis=-1, keepdims=True)
            if t < H:
                ks[t] = proj(t, 1).astype(bf16)
                vs[t] = proj(t, 2).astype(bf16)
            if t == 2:
                finalize(sp, slot)
            if t == H - 1:
                tbm = s // _NJ
                js = s % _NJ
                rows = pl.ds(pl.multiple_of(P + tbm * MB, 8), MB)
                xb = xn[rows, :]
                g = jax.lax.dot_general(xb, wg[js], dn, preferred_element_type=f32)
                u = jax.lax.dot_general(xb, wu[js], dn, preferred_element_type=f32)
            h = t - _SK2
            if 0 <= h < H:
                o = jax.lax.dot_general(es.pop(h), vs.pop(h), dn, preferred_element_type=f32)
                o40[:, h * E:(h + 1) * E] = o * ls.pop(h)
            if h in (H // 4, H // 2):
                part = wo_part(h // (H // 4) - 1)
                r = part if r is None else r + part
        r = r + wo_part(2)
        r = r + wo_part(3)
        h40[0:M, :] = r[0:M, :]
        sbuf[pl.ds(pl.multiple_of((s % 4) * SEG, SEG), SEG), :] = r[M:L, :]

        hb = jax.nn.sigmoid(g) * u
        d = jax.lax.dot_general(hb, wd[js], dn, preferred_element_type=f32)
        bacc[rows, :] = d + jnp.where(js > 0, bacc[rows, :], 0.0)

        @pl.when(s >= _LAG)
        def _():
            out_copy(sp, slot).start()

        return carry

    jax.lax.fori_loop(0, nseg, step, 0)
    for sp in range(nseg - _LAG, nseg):
        slot = sp % _NOB
        out_copy(sp - _NOB, slot).wait()
        finalize(sp, slot)
        out_copy(sp, slot).start()
    for sp in range(nseg - _NOB, nseg):
        out_copy(sp, sp % _NOB).wait()


@functools.partial(jax.jit, static_argnames=("A_seg_len",))
def pallas_recurrent_scan__memory_aug_recurrent_mem_tr__glu_gated_glu__prompt_kernel(
    A_x: jax.Array,
    A_mem0: jax.Array,
    A_Wq: jax.Array,
    A_Wk: jax.Array,
    A_Wv: jax.Array,
    A_Wo: jax.Array,
    A_seg_len: int,
    B_x: jax.Array,
    B_w_gate: jax.Array,
    B_w_up: jax.Array,
    B_w_down: jax.Array,
):
    B, S, D = A_x.shape
    assert B == 1
    _, H, E = A_Wq.shape
    M = A_mem0.shape[1]
    SEG = int(A_seg_len)
    F = B_w_gate.shape[1]
    L = M + SEG
    kern = functools.partial(_kernel, S=S, D=D, H=H, E=E, M=M, SEG=SEG, F=F)
    any_spec = pl.BlockSpec(memory_space=pl.ANY)
    out = pl.pallas_call(
        kern,
        out_shape=jax.ShapeDtypeStruct((S, D), A_x.dtype),
        in_specs=[any_spec, pl.BlockSpec(memory_space=pltpu.VMEM)] + [any_spec] * 7,
        out_specs=any_spec,
        scratch_shapes=[
            pltpu.VMEM((H * 3 * D // 2, E), jnp.uint32),
            pltpu.VMEM((H * E // 2, D), jnp.uint32),
            pltpu.VMEM((_NJ, D, F // _NJ), jnp.bfloat16),
            pltpu.VMEM((_NJ, D, F // _NJ), jnp.bfloat16),
            pltpu.VMEM((_NJ, F // _NJ, D), jnp.bfloat16),
            pltpu.VMEM((S, D), jnp.bfloat16),
            pltpu.VMEM((S, D), jnp.float32),
            pltpu.VMEM((_NSTG, 3, D // _NCH * H, E), jnp.bfloat16),
            pltpu.VMEM((_NSTG, H * E // _NCH, D), jnp.bfloat16),
            pltpu.VMEM((L, D), jnp.float32),
            pltpu.VMEM((L, H * E), jnp.float32),
            pltpu.VMEM((4 * SEG, D), jnp.float32),
            pltpu.VMEM((S, D), jnp.float32),
            pltpu.VMEM((_NOB, SEG, D), A_x.dtype),
            pltpu.SemaphoreType.DMA((3 * _NJ,)),
            pltpu.SemaphoreType.DMA(()),
            pltpu.SemaphoreType.DMA((_NSTG, 4)),
            pltpu.SemaphoreType.DMA((_NOB,)),
        ],
        compiler_params=pltpu.CompilerParams(vmem_limit_bytes=116 * 1024 * 1024),
        name="rmt_glu",
    )(
        A_x.reshape(S, D), A_mem0.reshape(M, D),
        A_Wq.reshape(D * H, E), A_Wk.reshape(D * H, E), A_Wv.reshape(D * H, E),
        A_Wo.reshape(H * E, D),
        B_w_gate, B_w_up, B_w_down,
    )
    return out.reshape(B, S, D)
```

```python
import functools

import jax
import jax.numpy as jnp
import jax.experimental.pallas as pl
import jax.experimental.pallas.tpu as pltpu

_PB = 128
_NPB = 6
_NJ = 4
_NCH = 16
_NSTG = 4
_LAG = 3
_NOB = 4
_SK1, _SK2 = 2, 4


def _kernel(x_hbm, mem0_ref, wq_hbm, wk_hbm, wv_hbm, wo_hbm, wg_hbm, wu_hbm, wd_hbm,
            out_hbm,
            wqkv, wo_i, wg, wu, wd, xv, xn, stg, stg2, h40, o40, sbuf, bacc, obuf,
            sem_b, sem_x, sem_s, sem_o, flag_ref,
            *, S, D, H, E, M, SEG, F):
    f32, bf16, u32 = jnp.float32, jnp.bfloat16, jnp.uint32
    L = M + SEG
    nseg = S // SEG
    FS = F // _NJ
    D2 = D // 2
    scale = E ** (-0.5)
    P = _PB * _NPB
    MB = (S - P) // (nseg // _NJ)
    DC = D // _NCH
    OC = H * E // _NCH
    dn = (((1,), (0,)), ((), ()))

    def b_copies(j):
        return [
            pltpu.make_async_copy(wg_hbm.at[:, pl.ds(j * FS, FS)], wg.at[j], sem_b.at[3 * j]),
            pltpu.make_async_copy(wu_hbm.at[:, pl.ds(j * FS, FS)], wu.at[j], sem_b.at[3 * j + 1]),
            pltpu.make_async_copy(wd_hbm.at[pl.ds(j * FS, FS), :], wd.at[j], sem_b.at[3 * j + 2]),
        ]

    def a_copies(c, slot):
        cps = []
        for j, src in enumerate((wq_hbm, wk_hbm, wv_hbm)):
            cps.append(pltpu.make_async_copy(src.at[pl.ds(pl.multiple_of(c * DC * H, DC * H), DC * H), :],
                                             stg.at[slot, j], sem_s.at[slot, j]))
        cps.append(pltpu.make_async_copy(wo_hbm.at[pl.ds(pl.multiple_of(c * OC, OC), OC), :],
                                         stg2.at[slot], sem_s.at[slot, 3]))
        return cps

    flag_ref[0] = nseg
    x_cp0 = pltpu.make_async_copy(x_hbm.at[pl.ds(0, P), :], xv.at[pl.ds(0, P), :], sem_x.at[0])
    x_cp1 = pltpu.make_async_copy(x_hbm.at[pl.ds(P, S - P), :], xv.at[pl.ds(P, S - P), :], sem_x.at[1])
    x_cp0.start()
    for cp in b_copies(0):
        cp.start()

    def ln(i, carry):
        r = pl.ds(pl.multiple_of(i * 64, 64), 64)
        xf = xv[r, :].astype(f32)
        m = jnp.mean(xf, axis=-1, keepdims=True)
        xc = xf - m
        v = jnp.mean(xc * xc, axis=-1, keepdims=True)
        xn[r, :] = xc * jax.lax.rsqrt(v + 1e-5)
        return carry

    x_cp0.wait()
    jax.lax.fori_loop(0, P // 64, ln, 0, unroll=2)

    def glu_chunk(rows, js, fillers=(), waits=(None, None, None)):
        fillers = list(fillers)
        nslot = 10
        per = -(-len(fillers) // nslot)
        always = js < flag_ref[0]
        pend = []

        def fill():
            for _ in range(min(per, len(fillers))):
                pend.extend(fillers.pop(0)())

        def tie(lhs):
            if not pend:
                return lhs
            nc = lhs.shape[1] // E
            vs = [pltpu.bitcast(v, f32) for v in pend]
            del pend[:]
            while len(vs) % nc:
                vs.append(vs[-1])
            bands = [jnp.concatenate(vs[i:i + nc], axis=1) for i in range(0, len(vs), nc)]
            nb = lhs.shape[0] // 8
            out = [lhs[8 * i:8 * i + 8] for i in range(nb)]
            for i, band in enumerate(bands):
                out[i % nb] = jnp.where(always, out[i % nb], band)
            return jnp.concatenate(out, axis=0)

        xb = xn[rows, :]
        nt = FS // E
        cuts = [0] + [min(nt, 2 * (i + 1)) * E for i in range((nt + 1) // 2)] if fillers else [0, (nt // 2 + 1) * E, FS]
        parts = list(zip(cuts[:-1], cuts[1:]))
        hs = []
        gs = []
        if waits[0] is not None:
            waits[0]()
        for lo, hi in parts:
            gs.append(jax.lax.dot_general(tie(xb), wg[js, :, lo:hi], dn, preferred_element_type=f32))
            fill()
        if waits[1] is not None:
            waits[1]()
        for (lo, hi), g in zip(parts, gs):
            u = jax.lax.dot_general(tie(xb), wu[js, :, lo:hi], dn, preferred_element_type=f32)
            hs.append(jax.nn.sigmoid(g) * u)
            fill()
        if waits[2] is not None:
            waits[2]()
        hb = jnp.concatenate(hs, axis=1)
        nd = 4 if fillers else 1
        dw = D // nd
        for i in range(nd):
            cols = slice(i * dw, (i + 1) * dw)
            d = jax.lax.dot_general(tie(hb), wd[js, :, cols], dn, preferred_element_type=f32)
            bacc[rows, cols] = d + jnp.where(js > 0, bacc[rows, cols], 0.0)
            if i + 1 < nd:
                fill()
        assert not fillers

    def relayout_units(c, slot):
        sub = jax.lax.broadcasted_iota(jnp.int32, (8, E), 0)

        def tr8(vs):
            vs = list(vs)
            for k in (1, 2, 4):
                m = (sub & k) == 0
                for i in range(8):
                    if i & k == 0:
                        a, b = vs[i], vs[i + k]
                        vs[i] = jnp.where(m, a, pltpu.roll(b, k, 0))
                        vs[i + k] = jnp.where(m, pltpu.roll(a, 8 - k, 0), b)
            return vs

        def qkv_unit(j, g, half):
            los, his = [], []
            for dp in range(8):
                r0 = (g * 16 + dp * 2) * H + half * 16
                a = pltpu.bitcast(stg[slot, j, pl.ds(r0, 16), :], u32)
                b = pltpu.bitcast(stg[slot, j, pl.ds(r0 + H, 16), :], u32)
                los.append((a & u32(0xFFFF)) | (b << 16))
                his.append((a >> 16) | (b & u32(0xFFFF0000)))
            los, his = tr8(los), tr8(his)
            for hp in range(8):
                h = half * 16 + 2 * hp
                base = (h * 3 + j) * D2 + g * 8
                wqkv[pl.ds(pl.multiple_of(base + c * (DC // 2), 8), 8), :] = los[hp]
                wqkv[pl.ds(pl.multiple_of(base + 3 * D2 + c * (DC // 2), 8), 8), :] = his[hp]
            return los + his

        def wo_unit(r):
            v = stg2[slot, pl.ds(r * 16, 16), :]
            wo_i[pl.ds(pl.multiple_of(c * (OC // 2) + r * 8, 8), 8), :] = pltpu.bitcast(v, u32)
            return []

        units = []
        for j in range(3):
            for g in range(DC // 16):
                for half in range(H // 16):
                    units.append(functools.partial(qkv_unit, j, g, half))
        wos = [functools.partial(wo_unit, r) for r in range(OC // 16)]
        mixed = []
        for i, un in enumerate(units):
            mixed.append(un)
            if i < len(wos):
                mixed.append(wos[i])
        return mixed + wos[len(units):]

    n_pro = _NPB * _NJ
    n_plain = n_pro - _NCH

    def wait_b(i):
        @pl.when(i % _NPB == 0)
        def _():
            for cp in b_copies(i // _NPB):
                cp.wait()

            @pl.when(i // _NPB + 1 < _NJ)
            def _():
                for cp in b_copies(i // _NPB + 1):
                    cp.start()

    def pro_plain(i, carry):
        wait_b(i)

        @pl.when(i == 2)
        def _():
            for c in range(_NSTG):
                for cp in a_copies(c, c):
                    cp.start()

        glu_chunk(pl.ds(pl.multiple_of((i % _NPB) * _PB, _PB), _PB), i // _NPB)
        return carry

    def pro_relayout(i, carry):
        wait_b(i)
        c = i - n_plain
        slot = c % _NSTG
        for cp in a_copies(c, slot):
            cp.wait()
        glu_chunk(pl.ds(pl.multiple_of((i % _NPB) * _PB, _PB), _PB), i // _NPB, relayout_units(c, slot))

        @pl.when(c + _NSTG < _NCH)
        def _():
            for cp in a_copies(c + _NSTG, slot):
                cp.start()
        return carry

    glu_chunk(pl.ds(0, _PB), 0, waits=[cp.wait for cp in b_copies(0)])
    for cp in b_copies(1):
        cp.start()
    jax.lax.fori_loop(1, n_plain, pro_plain, 0)
    x_cp1.start()
    jax.lax.fori_loop(n_plain, n_pro, pro_relayout, 0)

    x_cp1.wait()
    jax.lax.fori_loop(P // 64, S // 64, ln, 0, unroll=2)
    h40[0:M, :] = mem0_ref[...].astype(f32)
    sbuf[0:SEG, :] = jnp.zeros((SEG, D), f32)

    row = jax.lax.broadcasted_iota(jnp.int32, (L, L), 0)
    col = jax.lax.broadcasted_iota(jnp.int32, (L, L), 1)
    mask = (row < M) | (row >= col)

    def out_copy(sp, slot):
        return pltpu.make_async_copy(obuf.at[slot], out_hbm.at[pl.ds(pl.multiple_of(sp * SEG, SEG), SEG), :],
                                     sem_o.at[slot])

    def finalize(sp, slot):
        rows = pl.ds(pl.multiple_of(sp * SEG, SEG), SEG)
        b = bacc[rows, :]
        s_att = sbuf[pl.ds(pl.multiple_of((sp % 4) * SEG, SEG), SEG), :]
        res = xv[rows, :].astype(f32) + s_att * (b * jax.nn.sigmoid(b))
        obuf[slot] = res.astype(obuf.dtype)
        return res

    def step(s, carry):
        sp = jnp.maximum(s - _LAG, 0)
        slot = sp % _NOB

        @pl.when(s >= _LAG + _NOB)
        def _():
            out_copy(sp - _NOB, slot).wait()

        h40[M:L, :] = xn[pl.ds(pl.multiple_of(s * SEG, SEG), SEG), :]
        hh = h40[...]

        def proj(h, j):
            w = pltpu.bitcast(wqkv[(h * 3 + j) * D2:(h * 3 + j + 1) * D2, :], bf16)
            return jax.lax.dot_general(hh, w, dn, preferred_element_type=f32)

        def wo_part(i):
            n = H * E // 4
            return jax.lax.dot_general(o40[:, i * n:(i + 1) * n],
                                       pltpu.bitcast(wo_i[i * n // 2:(i + 1) * n // 2, :], bf16),
                                       dn, preferred_element_type=f32)

        qs, ks, vs, es, ls = {}, {}, {}, {}, {}

        def scores(h):
            sc = jax.lax.dot_general(qs.pop(h), ks.pop(h), (((1,), (1,)), ((), ())),
                                     preferred_element_type=f32) * scale
            sc = jnp.where(mask, sc, -1e9)
            e = jnp.exp(sc - jnp.max(sc, axis=-1, keepdims=True))
            es[h] = e
            ls[h] = 1.0 / jnp.sum(e, axis=-1, keepdims=True)

        def pv(h):
            o = jax.lax.dot_general(es.pop(h), vs.pop(h), dn, preferred_element_type=f32)
            o40[:, h * E:(h + 1) * E] = o * ls.pop(h)

        tbm = s // _NJ
        js = s % _NJ
        rows = pl.ds(pl.multiple_of(P + tbm * MB, 8), MB)
        always = s < flag_ref[0]
        r = None
        for t in range(H):
            qs[t] = proj(t, 0)
            if t >= _SK1:
                scores(t - _SK1)
            ks[t] = proj(t, 1).astype(bf16)
            vs[t] = proj(t, 2).astype(bf16)
            if t == 2:
                fin = finalize(sp, slot)
            if t == H - 1:
                xb = xn[rows, :]
                xb = jnp.concatenate([jnp.where(always, xb[:SEG], fin), xb[SEG:]], axis=0)
                g = jax.lax.dot_general(xb, wg[js], dn, preferred_element_type=f32)
                for h in range(H - _SK1, H):
                    scores(h)
            h = t - _SK2
            if h >= 0:
                pv(h)
            if h in (H // 4, H // 2):
                part = wo_part(h // (H // 4) - 1)
                r = part if r is None else r + part
        u = jax.lax.dot_general(xb, wu[js], dn, preferred_element_type=f32)
        for h in range(H - _SK2, H):
            pv(h)
        r = r + wo_part(2)
        r = r + wo_part(3)
        h40[0:M, :] = r[0:M, :]
        sbuf[pl.ds(pl.multiple_of((s % 4) * SEG, SEG), SEG), :] = r[M:L, :]

        hb = jax.nn.sigmoid(g) * u
        d = jax.lax.dot_general(hb, wd[js], dn, preferred_element_type=f32)
        bacc[rows, :] = d + jnp.where(js > 0, bacc[rows, :], 0.0)

        @pl.when(s >= _LAG)
        def _():
            out_copy(sp, slot).start()

        return carry

    jax.lax.fori_loop(0, nseg, step, 0)
    for sp in range(nseg - _LAG, nseg):
        slot = sp % _NOB
        out_copy(sp - _NOB, slot).wait()
        finalize(sp, slot)
        out_copy(sp, slot).start()
    for sp in range(nseg - _NOB, nseg):
        out_copy(sp, sp % _NOB).wait()


@functools.partial(jax.jit, static_argnames=("A_seg_len",))
def pallas_recurrent_scan__memory_aug_recurrent_mem_tr__glu_gated_glu__prompt_kernel(
    A_x: jax.Array,
    A_mem0: jax.Array,
    A_Wq: jax.Array,
    A_Wk: jax.Array,
    A_Wv: jax.Array,
    A_Wo: jax.Array,
    A_seg_len: int,
    B_x: jax.Array,
    B_w_gate: jax.Array,
    B_w_up: jax.Array,
    B_w_down: jax.Array,
):
    B, S, D = A_x.shape
    assert B == 1
    _, H, E = A_Wq.shape
    M = A_mem0.shape[1]
    SEG = int(A_seg_len)
    F = B_w_gate.shape[1]
    L = M + SEG
    kern = functools.partial(_kernel, S=S, D=D, H=H, E=E, M=M, SEG=SEG, F=F)
    any_spec = pl.BlockSpec(memory_space=pl.ANY)
    out = pl.pallas_call(
        kern,
        out_shape=jax.ShapeDtypeStruct((S, D), A_x.dtype),
        in_specs=[any_spec, pl.BlockSpec(memory_space=pltpu.VMEM)] + [any_spec] * 7,
        out_specs=any_spec,
        scratch_shapes=[
            pltpu.VMEM((H * 3 * D // 2, E), jnp.uint32),
            pltpu.VMEM((H * E // 2, D), jnp.uint32),
            pltpu.VMEM((_NJ, D, F // _NJ), jnp.bfloat16),
            pltpu.VMEM((_NJ, D, F // _NJ), jnp.bfloat16),
            pltpu.VMEM((_NJ, F // _NJ, D), jnp.bfloat16),
            pltpu.VMEM((S, D), jnp.bfloat16),
            pltpu.VMEM((S, D), jnp.float32),
            pltpu.VMEM((_NSTG, 3, D // _NCH * H, E), jnp.bfloat16),
            pltpu.VMEM((_NSTG, H * E // _NCH, D), jnp.bfloat16),
            pltpu.VMEM((L, D), jnp.float32),
            pltpu.VMEM((L, H * E), jnp.float32),
            pltpu.VMEM((4 * SEG, D), jnp.float32),
            pltpu.VMEM((S, D), jnp.float32),
            pltpu.VMEM((_NOB, SEG, D), A_x.dtype),
            pltpu.SemaphoreType.DMA((3 * _NJ,)),
            pltpu.SemaphoreType.DMA((2,)),
            pltpu.SemaphoreType.DMA((_NSTG, 4)),
            pltpu.SemaphoreType.DMA((_NOB,)),
            pltpu.SMEM((1,), jnp.int32),
        ],
        compiler_params=pltpu.CompilerParams(vmem_limit_bytes=116 * 1024 * 1024),
        name="rmt_glu",
    )(
        A_x.reshape(S, D), A_mem0.reshape(M, D),
        A_Wq.reshape(D * H, E), A_Wk.reshape(D * H, E), A_Wv.reshape(D * H, E),
        A_Wo.reshape(H * E, D),
        B_w_gate, B_w_up, B_w_down,
    )
    return out.reshape(B, S, D)
```
